```python
import os as _os
_os.environ.setdefault('JAX_PLATFORMS', 'cpu')
import jax
import jax.numpy as jnp

def _softmax(x, axis=-1):
    return jax.nn.softmax(x, axis=axis)

def _gelu(x):
    return jax.nn.gelu(x, approximate=True)

def _silu(x):
    return jax.nn.silu(x)

def _sigmoid(x):
    return jax.nn.sigmoid(x)

def _layernorm(x, axis=-1, eps=1e-05):
    m = jnp.mean(x, axis=axis, keepdims=True)
    v = jnp.var(x, axis=axis, keepdims=True)
    return (x - m) / jnp.sqrt(v + eps)

def _scatter_add(tgt, idx, src, axis=0):
    return tgt.at[idx].add(src)

def _segment_sum(src, seg, n):
    return jax.ops.segment_sum(src, seg, n)

class _Rng:

    def __init__(self, key):
        self._k = key

    def _next(self):
        self._k, sub = jax.random.split(self._k)
        return sub

    def normal(self, shape):
        return jax.random.normal(self._next(), shape, dtype=jnp.bfloat16)

    def randint(self, lo, hi, shape):
        return jax.random.randint(self._next(), shape, lo, hi, dtype=jnp.int32)

    def uniform(self, shape, lo=0.0, hi=1.0):
        return jax.random.uniform(self._next(), shape, jnp.bfloat16, lo, hi)

    def permutation(self, n):
        return jax.random.permutation(self._next(), n)
kernel_name = 'adaLN_cond__mha_block__dense_activation_squared_relu__prompt'

def setup_inputs():
    _rng = _Rng(jax.random.key(int.from_bytes(__import__("os").urandom(4), "little")))
    _w = lambda a: (lambda t: t.astype(jnp.bfloat16) if jnp.issubdtype(t.dtype, jnp.floating) else t)(jnp.asarray(a))

    def _A_setup():
        B, S, D, H = (1, 2048, 512, 32)
        return {'x': _w((lambda *s: _rng.normal(s) * 0.05)(B, S, D)), 'wqkv': _w((lambda *s: _rng.normal(s) * 0.1)(D, 3 * D)), 'wo': _w((lambda *s: _rng.normal(s) * 0.05)(D, D))}
    _A_in = _A_setup()

    def _B_setup():
        B, S, D, F = (1, 2048, 512, 1792)
        return {'x': _w((lambda *s: _rng.normal(s) * 0.05)(B, S, D)), 'w1': _w((lambda *s: _rng.normal(s) * 0.05)(D, F)), 'b1': _w((lambda *s: _rng.normal(s) * 0.05)(F)), 'w2': _w((lambda *s: _rng.normal(s) * 0.05)(F, D)), 'b2': _w((lambda *s: _rng.normal(s) * 0.05)(D))}
    _B_in = _B_setup()
    return {'A_x': _A_in['x'], 'A_wqkv': _A_in['wqkv'], 'A_wo': _A_in['wo'], 'B_x': _B_in['x'], 'B_w1': _B_in['w1'], 'B_b1': _B_in['b1'], 'B_w2': _B_in['w2'], 'B_b2': _B_in['b2'], 'c': _w((lambda *s: _rng.normal(s) * 0.05)(1, 512) * 8.0), 'w_mod': _w((lambda *s: _rng.normal(s) * 0.05)(512, 6 * 512) * 512 ** (-0.5) * 8.0)}

def reference(A_x, A_wqkv, A_wo, B_x, B_w1, B_b1, B_w2, B_b2, c, w_mod):

    def _A_ref(x, wqkv, wo):
        B, S, D = x.shape
        H = 32
        Dh = D // H
        qkv = (lambda x, *d: x.transpose(*d))((x @ wqkv).reshape(B, S, 3, H, Dh), 2, 0, 3, 1, 4)
        q, k, v = (qkv[0], qkv[1], qkv[2])
        scores = jnp.einsum('bhqd,bhkd->bhqk', q, k) * Dh ** (-0.5)
        p = _softmax(scores, axis=-1)
        o = jnp.einsum('bhqk,bhkd->bhqd', p, v)
        return (lambda x, *d: x.transpose(*d))(o, 0, 2, 1, 3).reshape(B, S, D) @ wo

    def _B_ref(x, w1, b1, w2, b2):
        h = jnp.einsum('bsd,df->bsf', x, w1) + b1
        zero = jnp.zeros_like(h)
        r = jnp.where(h > zero, h, zero)
        h = r * r
        out = jnp.einsum('bsf,fd->bsd', h, w2) + b2
        return out
    x = A_x
    mod = (_silu(c) @ w_mod).reshape(c.shape[0], 6, 1, -1)
    sa, ca, ga, sb, cb, gb = (mod[:, 0].copy(), mod[:, 1].copy(), mod[:, 2].copy(), mod[:, 3].copy(), mod[:, 4].copy(), mod[:, 5].copy())
    h = _layernorm(x, axis=-1) * (1 + ca) + sa
    x = x + ga * _A_ref(h, A_wqkv, A_wo)
    h = _layernorm(x, axis=-1) * (1 + cb) + sb
    x = x + gb * _B_ref(h, B_w1, B_b1, B_w2, B_b2)
    return x
```

```python
import functools

import jax
import jax.numpy as jnp
import numpy as np
from jax import lax
import jax.experimental.pallas as pl
import jax.experimental.pallas.tpu as pltpu

_BF = jnp.bfloat16
_F32 = jnp.float32
_LOG2E = float(np.log2(np.e))
_EPS = 1e-5

_H = 32
_TQ = 512
_KC = 128
_G = 128


def _layernorm(x):
    m = jnp.mean(x, axis=-1, keepdims=True)
    xc = x - m
    v = jnp.mean(xc * xc, axis=-1, keepdims=True)
    return xc * lax.rsqrt(v + _EPS)


def _kernel(x_hbm, wqkv_hbm, wo_hbm, w1_hbm, b1_hbm, w2_hbm, b2_hbm, c_hbm, wmod_hbm,
            o_ref,
            x_s, wqkv_s, wo_s, w1_s, b1_s, w2_s, b2_s, c_s, wmod_s, mod_s,
            qt_s, k_s, vt_s, ot_s, s0, s1, sems, *, S, D):
    i = pl.program_id(0)
    Dh = D // _H
    NT = S // _TQ
    NG = D // _G
    HPG = _G // Dh
    NC = S // _KC

    copies = [
        pltpu.make_async_copy(c_hbm, c_s, sems.at[0]),
        pltpu.make_async_copy(wmod_hbm, wmod_s, sems.at[1]),
        pltpu.make_async_copy(x_hbm, x_s, sems.at[2]),
        pltpu.make_async_copy(wqkv_hbm, wqkv_s, sems.at[3]),
        pltpu.make_async_copy(wo_hbm, wo_s, sems.at[4]),
        pltpu.make_async_copy(w1_hbm, w1_s, sems.at[5]),
        pltpu.make_async_copy(b1_hbm, b1_s, sems.at[6]),
        pltpu.make_async_copy(w2_hbm, w2_s, sems.at[7]),
        pltpu.make_async_copy(b2_hbm, b2_s, sems.at[8]),
    ]

    def mod(j):
        return mod_s[0:1, j * D:(j + 1) * D]

    @pl.when(i == 0)
    def _prologue():
        for cp in copies[:4]:
            cp.start()
        copies[0].wait()
        copies[1].wait()
        cv = c_s[...].astype(_F32)
        sc = (cv * jax.nn.sigmoid(cv)).astype(_BF)
        sc = jnp.broadcast_to(sc, (16, D))
        mod_s[...] = jnp.dot(sc, wmod_s[...], preferred_element_type=_F32)[0:8]
        copies[2].wait()
        copies[3].wait()
        for cp in copies[4:]:
            cp.start()

        def qkv_body(t, _):
            r0 = pl.multiple_of(t * _TQ, _TQ)
            xr = x_s[pl.ds(r0, _TQ), :].astype(_F32)
            h = (_layernorm(xr) * (1.0 + mod(1)) + mod(0)).astype(_BF)
            q = jnp.dot(h, wqkv_s[:, 0:D], preferred_element_type=_F32)
            q = q * (Dh ** -0.5 * _LOG2E)
            qt_s[t] = q.T.astype(_BF)
            k = jnp.dot(h, wqkv_s[:, D:2 * D], preferred_element_type=_F32).astype(_BF)
            for g in range(NG):
                k_s[g, pl.ds(r0, _TQ), :] = k[:, g * _G:(g + 1) * _G]
            v = jnp.dot(h, wqkv_s[:, 2 * D:3 * D], preferred_element_type=_F32)
            vt_s[:, pl.ds(r0, _TQ)] = v.T.astype(_BF)
            return 0
        lax.fori_loop(0, NT, qkv_body, 0)

        rowhead = lax.broadcasted_iota(jnp.int32, (_G, _TQ), 0) // Dh

        def item(n):
            return n // _H, n % _H

        def qmask(n):
            t, h = item(n)
            g = h // HPG
            q = qt_s[t, pl.ds(pl.multiple_of(g * _G, _G), _G), :]
            return jnp.where(rowhead == h % HPG, q, jnp.zeros_like(q))

        def stage_a(n, c, qm, sbuf, m8):
            _, h = item(n)
            s = jnp.dot(k_s[h // HPG, c * _KC:(c + 1) * _KC, :], qm, preferred_element_type=_F32)
            sbuf[c * _KC:(c + 1) * _KC, :] = s
            mm = jnp.max(s.reshape(_KC // 8, 8, _TQ), axis=0)
            return mm if m8 is None else jnp.maximum(m8, mm)

        def stage_b(n, c, sbuf, m, acc, l8):
            _, h = item(n)
            p = jnp.exp2(sbuf[c * _KC:(c + 1) * _KC, :] - m)
            ls = jnp.sum(p.reshape(_KC // 8, 8, _TQ), axis=0)
            v = vt_s[pl.ds(pl.multiple_of(h * Dh, Dh), Dh), c * _KC:(c + 1) * _KC]
            r = jnp.dot(v, p.astype(_BF), preferred_element_type=_F32)
            if acc is None:
                return r, ls
            return acc + r, l8 + ls

        def finish(n, acc, l8):
            t, h = item(n)
            l = jnp.sum(l8, axis=0, keepdims=True)
            o = acc * pl.reciprocal(l, approx=False)
            ot_s[t, pl.ds(pl.multiple_of(h * Dh, Dh), Dh), :] = o.astype(_BF)

        def step(na, sa, nb, sb, mb):
            qm = qmask(na) if na is not None else None
            m8 = acc = l8 = None
            for c in range(NC):
                if na is not None:
                    m8 = stage_a(na, c, qm, sa, m8)
                if nb is not None:
                    acc, l8 = stage_b(nb, c, sb, mb, acc, l8)
            if nb is not None:
                finish(nb, acc, l8)
            if na is not None:
                return jnp.max(m8, axis=0, keepdims=True)
            return None

        NI = NT * _H
        m0 = step(0, s0, None, None, None)

        def body(j, m):
            m = step(2 * j + 1, s1, 2 * j, s0, m)
            m = step(2 * j + 2, s0, 2 * j + 1, s1, m)
            return m
        m = lax.fori_loop(0, NI // 2 - 1, body, m0)
        m = step(NI - 1, s1, NI - 2, s0, m)
        step(None, None, NI - 1, s1, m)

        for cp in copies[4:]:
            cp.wait()

    r0 = pl.multiple_of(i * _TQ, _TQ)
    xr = x_s[pl.ds(r0, _TQ), :].astype(_F32)
    a = lax.dot_general(ot_s[i], wo_s[...], (((0,), (0,)), ((), ())), preferred_element_type=_F32)
    x1 = xr + mod(2) * a
    h = (_layernorm(x1) * (1.0 + mod(4)) + mod(3)).astype(_BF)
    f = jnp.dot(h, w1_s[...], preferred_element_type=_F32) + b1_s[...].astype(_F32)
    f = jnp.maximum(f, 0.0)
    f = (f * f).astype(_BF)
    y = jnp.dot(f, w2_s[...], preferred_element_type=_F32) + b2_s[...].astype(_F32)
    o_ref[...] = (x1 + mod(5) * y).astype(o_ref.dtype)


@jax.jit
def pallas_adaLN_cond__mha_block__dense_activation_squared_relu__prompt_kernel(
    A_x: jax.Array,
    A_wqkv: jax.Array,
    A_wo: jax.Array,
    B_x: jax.Array,
    B_w1: jax.Array,
    B_b1: jax.Array,
    B_w2: jax.Array,
    B_b2: jax.Array,
    c: jax.Array,
    w_mod: jax.Array,
):
    del B_x
    B, S, D = A_x.shape
    F = B_w1.shape[1]
    assert B == 1
    x2 = A_x.reshape(S, D)
    any_spec = pl.BlockSpec(memory_space=pl.ANY)
    out = pl.pallas_call(
        functools.partial(_kernel, S=S, D=D),
        grid=(S // _TQ,),
        in_specs=[any_spec] * 9,
        out_specs=pl.BlockSpec((_TQ, D), lambda i: (i, 0)),
        out_shape=jax.ShapeDtypeStruct((S, D), A_x.dtype),
        scratch_shapes=[
            pltpu.VMEM((S, D), A_x.dtype),
            pltpu.VMEM((D, 3 * D), A_wqkv.dtype),
            pltpu.VMEM((D, D), A_wo.dtype),
            pltpu.VMEM((D, F), B_w1.dtype),
            pltpu.VMEM((1, F), B_b1.dtype),
            pltpu.VMEM((F, D), B_w2.dtype),
            pltpu.VMEM((1, D), B_b2.dtype),
            pltpu.VMEM((1, D), c.dtype),
            pltpu.VMEM((D, 6 * D), w_mod.dtype),
            pltpu.VMEM((8, 6 * D), _F32),
            pltpu.VMEM((S // _TQ, D, _TQ), _BF),
            pltpu.VMEM((D // _G, S, _G), _BF),
            pltpu.VMEM((D, S), _BF),
            pltpu.VMEM((S // _TQ, D, _TQ), _BF),
            pltpu.VMEM((S, _TQ), _F32),
            pltpu.VMEM((S, _TQ), _F32),
            pltpu.SemaphoreType.DMA((9,)),
        ],
        compiler_params=pltpu.CompilerParams(
            dimension_semantics=("arbitrary",),
            vmem_limit_bytes=110 * 1024 * 1024,
        ),
    )(x2, A_wqkv, A_wo, B_w1, B_b1.reshape(1, F), B_w2, B_b2.reshape(1, D), c, w_mod)
    return out.reshape(B, S, D)
```

```python
import functools

import jax
import jax.numpy as jnp
import numpy as np
from jax import lax
import jax.experimental.pallas as pl
import jax.experimental.pallas.tpu as pltpu

_BF = jnp.bfloat16
_F32 = jnp.float32
_LOG2E = float(np.log2(np.e))
_EPS = 1e-5

_H = 32
_TQ = 512
_KC = 128
_KX = 256
_G = 128


def _layernorm(x):
    m = jnp.mean(x, axis=-1, keepdims=True)
    xc = x - m
    v = jnp.mean(xc * xc, axis=-1, keepdims=True)
    return xc * lax.rsqrt(v + _EPS)


def _kernel(x_hbm, wqkv_hbm, wo_hbm, w1_hbm, b1_hbm, w2_hbm, b2_hbm, c_hbm, wmod_hbm,
            o_ref,
            x_s, wqkv_s, wo_s, w1_s, b1_s, w2_s, b2_s, c_s, wmod_s, mod_s,
            qt_s, k_s, vt_s, ot_s, sems, *, S, D):
    i = pl.program_id(0)
    Dh = D // _H
    NT = S // _TQ
    NG = D // _G
    HPG = _G // Dh
    NC = S // _KC

    copies = [
        pltpu.make_async_copy(c_hbm, c_s, sems.at[0]),
        pltpu.make_async_copy(wmod_hbm, wmod_s, sems.at[1]),
        pltpu.make_async_copy(x_hbm, x_s, sems.at[2]),
        pltpu.make_async_copy(wqkv_hbm, wqkv_s, sems.at[3]),
        pltpu.make_async_copy(wo_hbm, wo_s, sems.at[4]),
        pltpu.make_async_copy(w1_hbm, w1_s, sems.at[5]),
        pltpu.make_async_copy(b1_hbm, b1_s, sems.at[6]),
        pltpu.make_async_copy(w2_hbm, w2_s, sems.at[7]),
        pltpu.make_async_copy(b2_hbm, b2_s, sems.at[8]),
    ]

    def mod(j):
        return mod_s[0:1, j * D:(j + 1) * D]

    @pl.when(i == 0)
    def _prologue():
        for cp in copies[:4]:
            cp.start()
        copies[0].wait()
        copies[1].wait()
        cv = c_s[...].astype(_F32)
        sc = (cv * jax.nn.sigmoid(cv)).astype(_BF)
        sc = jnp.broadcast_to(sc, (16, D))
        mod_s[...] = jnp.dot(sc, wmod_s[...], preferred_element_type=_F32)[0:8]
        copies[2].wait()
        copies[3].wait()
        for cp in copies[4:]:
            cp.start()

        def qkv_body(t, _):
            r0 = pl.multiple_of(t * _TQ, _TQ)
            xr = x_s[pl.ds(r0, _TQ), :].astype(_F32)
            h = (_layernorm(xr) * (1.0 + mod(1)) + mod(0)).astype(_BF)
            q = jnp.dot(h, wqkv_s[:, 0:D], preferred_element_type=_F32)
            q = q * (Dh ** -0.5 * _LOG2E)
            qt_s[pl.ds(t * NG, NG)] = q.T.astype(_BF).reshape(NG, _G, _TQ)
            k = jnp.dot(h, wqkv_s[:, D:2 * D], preferred_element_type=_F32).astype(_BF)
            for g in range(NG):
                k_s[g, pl.ds(r0, _TQ), :] = k[:, g * _G:(g + 1) * _G]
            v = jnp.dot(h, wqkv_s[:, 2 * D:3 * D], preferred_element_type=_F32)
            vt = v.T.astype(_BF)
            for g in range(NG):
                vt_s[g, :, pl.ds(r0, _TQ)] = vt[g * _G:(g + 1) * _G]
            return 0
        lax.fori_loop(0, NT, qkv_body, 0)

        def attn_body(n, carry):
            lmax, lmin = carry
            g = n % NG
            seq = [(i, c) for i in range(HPG) for c in range(NC)]
            qm, sv, pv, acc, l8 = {}, {}, {}, {}, {}
            for u in range(len(seq) + 2):
                if u < len(seq):
                    i, c = seq[u]
                    if c == 0:
                        parts = [qt_s[n, i * Dh:(i + 1) * Dh, :]]
                        if i > 0:
                            parts = [jnp.zeros((i * Dh, _TQ), _BF)] + parts
                        if i < HPG - 1:
                            parts = parts + [jnp.zeros((_G - (i + 1) * Dh, _TQ), _BF)]
                        qm[i] = jnp.concatenate(parts, axis=0)
                    sv[u] = jnp.dot(k_s[g, c * _KC:(c + 1) * _KC, :], qm[i],
                                    preferred_element_type=_F32)
                if 0 <= u - 1 < len(seq):
                    i, c = seq[u - 1]
                    s = sv.pop(u - 1)
                    ps, ls = [], None
                    for r in range(_KC // 16):
                        p = jnp.exp2(s[r * 16:(r + 1) * 16])
                        t2 = p[0:8] + p[8:16]
                        ls = t2 if ls is None else ls + t2
                        ps.append(p.astype(_BF))
                    pv[u - 1] = jnp.concatenate(ps, axis=0)
                    l8[i] = ls if c == 0 else l8[i] + ls
                if u - 2 >= 0:
                    i, c = seq[u - 2]
                    v = vt_s[g, i * Dh:(i + 1) * Dh, c * _KC:(c + 1) * _KC]
                    r = jnp.dot(v, pv.pop(u - 2), preferred_element_type=_F32)
                    acc[i] = r if c == 0 else acc[i] + r
                    if c == NC - 1:
                        l = jnp.sum(l8[i], axis=0, keepdims=True)
                        lmax = jnp.maximum(lmax, l)
                        lmin = jnp.minimum(lmin, l)
                        o = acc[i] * pl.reciprocal(l, approx=False)
                        ot_s[n, i * Dh:(i + 1) * Dh, :] = o.astype(_BF)
            return lmax, lmin

        lmax, lmin = lax.fori_loop(
            0, NT * NG, attn_body,
            (jnp.ones((1, _TQ), _F32), jnp.ones((1, _TQ), _F32)))
        ok = jnp.logical_and(lmax <= 2.0 ** 100, lmin >= 2.0 ** -60)
        n_bad = jnp.sum(jnp.where(ok, 0.0, 1.0))

        @pl.when(n_bad > 0.0)
        def _exact_attention():
            rowhead = lax.broadcasted_iota(jnp.int32, (_G, _TQ), 0) // Dh

            def item(j, _):
                n = j // HPG
                i = j % HPG
                g = n % NG
                q = qt_s[n]
                q = jnp.where(rowhead == i, q, jnp.zeros_like(q))
                r16 = pl.ds(pl.multiple_of(i * Dh, Dh), Dh)

                def chunk(c, carry):
                    m, l, a = carry
                    ck = pl.ds(pl.multiple_of(c * _KX, _KX), _KX)
                    s = jnp.dot(k_s[g, ck, :], q, preferred_element_type=_F32)
                    mn = jnp.maximum(m, jnp.max(s, axis=0, keepdims=True))
                    al = jnp.exp2(m - mn)
                    p = jnp.exp2(s - mn)
                    l = l * al + jnp.sum(p, axis=0, keepdims=True)
                    a = a * al + jnp.dot(vt_s[g, r16, ck], p.astype(_BF),
                                         preferred_element_type=_F32)
                    return mn, l, a
                m, l, a = lax.fori_loop(
                    0, S // _KX, chunk,
                    (jnp.full((1, _TQ), -jnp.inf, _F32), jnp.zeros((1, _TQ), _F32),
                     jnp.zeros((Dh, _TQ), _F32)))
                ot_s[n, r16, :] = (a * pl.reciprocal(l, approx=False)).astype(_BF)
                return 0
            lax.fori_loop(0, NT * _H, item, 0)

        for cp in copies[4:]:
            cp.wait()

    r0 = pl.multiple_of(i * _TQ, _TQ)
    xr = x_s[pl.ds(r0, _TQ), :].astype(_F32)
    ot = ot_s[pl.ds(i * NG, NG)].reshape(D, _TQ)
    a = lax.dot_general(ot, wo_s[...], (((0,), (0,)), ((), ())), preferred_element_type=_F32)
    x1 = xr + mod(2) * a
    h = (_layernorm(x1) * (1.0 + mod(4)) + mod(3)).astype(_BF)
    f = jnp.dot(h, w1_s[...], preferred_element_type=_F32) + b1_s[...].astype(_F32)
    f = jnp.maximum(f, 0.0)
    f = (f * f).astype(_BF)
    y = jnp.dot(f, w2_s[...], preferred_element_type=_F32) + b2_s[...].astype(_F32)
    o_ref[...] = (x1 + mod(5) * y).astype(o_ref.dtype)


@jax.jit
def pallas_adaLN_cond__mha_block__dense_activation_squared_relu__prompt_kernel(
    A_x: jax.Array,
    A_wqkv: jax.Array,
    A_wo: jax.Array,
    B_x: jax.Array,
    B_w1: jax.Array,
    B_b1: jax.Array,
    B_w2: jax.Array,
    B_b2: jax.Array,
    c: jax.Array,
    w_mod: jax.Array,
):
    del B_x
    B, S, D = A_x.shape
    F = B_w1.shape[1]
    assert B == 1
    x2 = A_x.reshape(S, D)
    any_spec = pl.BlockSpec(memory_space=pl.ANY)
    out = pl.pallas_call(
        functools.partial(_kernel, S=S, D=D),
        grid=(S // _TQ,),
        in_specs=[any_spec] * 9,
        out_specs=pl.BlockSpec((_TQ, D), lambda i: (i, 0)),
        out_shape=jax.ShapeDtypeStruct((S, D), A_x.dtype),
        scratch_shapes=[
            pltpu.VMEM((S, D), A_x.dtype),
            pltpu.VMEM((D, 3 * D), A_wqkv.dtype),
            pltpu.VMEM((D, D), A_wo.dtype),
            pltpu.VMEM((D, F), B_w1.dtype),
            pltpu.VMEM((1, F), B_b1.dtype),
            pltpu.VMEM((F, D), B_w2.dtype),
            pltpu.VMEM((1, D), B_b2.dtype),
            pltpu.VMEM((1, D), c.dtype),
            pltpu.VMEM((D, 6 * D), w_mod.dtype),
            pltpu.VMEM((8, 6 * D), _F32),
            pltpu.VMEM((S // _TQ * D // _G, _G, _TQ), _BF),
            pltpu.VMEM((D // _G, S, _G), _BF),
            pltpu.VMEM((D // _G, _G, S), _BF),
            pltpu.VMEM((S // _TQ * D // _G, _G, _TQ), _BF),
            pltpu.SemaphoreType.DMA((9,)),
        ],
        compiler_params=pltpu.CompilerParams(
            dimension_semantics=("arbitrary",),
            vmem_limit_bytes=110 * 1024 * 1024,
        ),
    )(x2, A_wqkv, A_wo, B_w1, B_b1.reshape(1, F), B_w2, B_b2.reshape(1, D), c, w_mod)
    return out.reshape(B, S, D)
```

```python
import functools

import jax
import jax.numpy as jnp
import numpy as np
from jax import lax
import jax.experimental.pallas as pl
import jax.experimental.pallas.tpu as pltpu

_BF = jnp.bfloat16
_F32 = jnp.float32
_LOG2E = float(np.log2(np.e))
_EPS = 1e-5

_H = 32
_TQ = 512
_TR = 256
_KC = 128
_KX = 256
_G = 128


def _layernorm(x):
    m = jnp.mean(x, axis=-1, keepdims=True)
    xc = x - m
    v = jnp.mean(xc * xc, axis=-1, keepdims=True)
    return xc * lax.rsqrt(v + _EPS)


def _kernel(x_hbm, wqkv_hbm, wo_hbm, w1_hbm, b1_hbm, w2_hbm, b2_hbm, c_hbm, wmod_hbm,
            o_hbm,
            x_s, wqkv_s, wo_s, w1_s, b1_s, w2_s, b2_s, c_s, wmod_s, mod_s,
            qt_s, k_s, vt_s, ot_s, out_s, sems, osems, *, S, D):
    Dh = D // _H
    NT = S // _TQ
    NG = D // _G
    HPG = _G // Dh
    NC = S // _KC
    NR = S // _TR

    def rows(t, n):
        return pl.ds(t * n, n)

    cp_c = pltpu.make_async_copy(c_hbm, c_s, sems.at[0])
    cp_mod = [pltpu.make_async_copy(wmod_hbm.at[:, j * 2 * D:(j + 1) * 2 * D], wmod_s.at[j], sems.at[1 + j])
              for j in range(3)]
    cp_qkv = [pltpu.make_async_copy(wqkv_hbm.at[:, j * D:(j + 1) * D], wqkv_s.at[j], sems.at[4 + j])
              for j in range(3)]
    cp_x = [pltpu.make_async_copy(x_hbm.at[rows(t, _TQ)], x_s.at[rows(t, _TQ)], sems.at[7 + t])
            for t in range(NT)]
    cp_rest = [
        pltpu.make_async_copy(wo_hbm, wo_s, sems.at[7 + NT]),
        pltpu.make_async_copy(w1_hbm, w1_s, sems.at[8 + NT]),
        pltpu.make_async_copy(b1_hbm, b1_s, sems.at[9 + NT]),
        pltpu.make_async_copy(w2_hbm, w2_s, sems.at[10 + NT]),
        pltpu.make_async_copy(b2_hbm, b2_s, sems.at[11 + NT]),
    ]

    def mod(j):
        return mod_s[0:1, j * D:(j + 1) * D]

    for cp in [cp_c, cp_mod[0], cp_x[0]] + cp_qkv:
        cp.start()
    cp_c.wait()
    cv = c_s[...].astype(_F32)
    sc = jnp.broadcast_to((cv * jax.nn.sigmoid(cv)).astype(_BF), (16, D))

    def modulation(j):
        cp_mod[j].wait()
        mod_s[:, j * 2 * D:(j + 1) * 2 * D] = jnp.dot(
            sc, wmod_s[j], preferred_element_type=_F32)[0:8]

    modulation(0)

    def ln1(t):
        cp_x[t].wait()
        xr = x_s[rows(t, _TQ), :].astype(_F32)
        return (_layernorm(xr) * (1.0 + mod(1)) + mod(0)).astype(_BF)

    hn = ln1(0)
    for t in range(NT):
        h = hn
        if t == 0:
            cp_qkv[0].wait()
        q = jnp.dot(h, wqkv_s[0], preferred_element_type=_F32)
        if t == 0:
            cp_qkv[1].wait()
        k = jnp.dot(h, wqkv_s[1], preferred_element_type=_F32)
        if t == 0:
            cp_qkv[2].wait()
            for cp in cp_x[1:] + cp_mod[1:]:
                cp.start()
        v = jnp.dot(h, wqkv_s[2], preferred_element_type=_F32)
        if t == 1:
            for cp in cp_rest:
                cp.start()
        q = q * (Dh ** -0.5 * _LOG2E)
        qt_s[pl.ds(t * NG, NG)] = q.T.astype(_BF).reshape(NG, _G, _TQ)
        if t + 1 < NT:
            hn = ln1(t + 1)
        k = k.astype(_BF)
        for g in range(NG):
            k_s[g, rows(t, _TQ), :] = k[:, g * _G:(g + 1) * _G]
        vt = v.T.astype(_BF)
        for g in range(NG):
            vt_s[g, :, rows(t, _TQ)] = vt[g * _G:(g + 1) * _G]
    modulation(1)
    modulation(2)

    def attn_body(n, carry):
        lmax, lmin = carry
        g = n % NG
        seq = [(i, c) for i in range(HPG) for c in range(NC)]
        qm, sv, pv, acc, l8 = {}, {}, {}, {}, {}
        for u in range(len(seq) + 2):
            if u < len(seq):
                i, c = seq[u]
                if c == 0:
                    parts = [qt_s[n, i * Dh:(i + 1) * Dh, :]]
                    if i > 0:
                        parts = [jnp.zeros((i * Dh, _TQ), _BF)] + parts
                    if i < HPG - 1:
                        parts = parts + [jnp.zeros((_G - (i + 1) * Dh, _TQ), _BF)]
                    qm[i] = jnp.concatenate(parts, axis=0)
                sv[u] = jnp.dot(k_s[g, c * _KC:(c + 1) * _KC, :], qm[i],
                                preferred_element_type=_F32)
            if 0 <= u - 1 < len(seq):
                i, c = seq[u - 1]
                s = sv.pop(u - 1)
                ps, ls = [], None
                for r in range(_KC // 16):
                    p = jnp.exp2(s[r * 16:(r + 1) * 16])
                    t2 = p[0:8] + p[8:16]
                    ls = t2 if ls is None else ls + t2
                    ps.append(p.astype(_BF))
                pv[u - 1] = jnp.concatenate(ps, axis=0)
                l8[i] = ls if c == 0 else l8[i] + ls
            if u - 2 >= 0:
                i, c = seq[u - 2]
                v = vt_s[g, i * Dh:(i + 1) * Dh, c * _KC:(c + 1) * _KC]
                r = jnp.dot(v, pv.pop(u - 2), preferred_element_type=_F32)
                acc[i] = r if c == 0 else acc[i] + r
                if c == NC - 1:
                    l = jnp.sum(l8[i], axis=0, keepdims=True)
                    lmax = jnp.maximum(lmax, l)
                    lmin = jnp.minimum(lmin, l)
                    o = acc[i] * pl.reciprocal(l, approx=False)
                    ot_s[n, i * Dh:(i + 1) * Dh, :] = o.astype(_BF)
        return lmax, lmin

    lmax, lmin = lax.fori_loop(
        0, NT * NG, attn_body,
        (jnp.ones((1, _TQ), _F32), jnp.ones((1, _TQ), _F32)))
    ok = jnp.logical_and(lmax <= 2.0 ** 100, lmin >= 2.0 ** -60)
    n_bad = jnp.sum(jnp.where(ok, 0.0, 1.0))

    @pl.when(n_bad > 0.0)
    def _exact_attention():
        rowhead = lax.broadcasted_iota(jnp.int32, (_G, _TQ), 0) // Dh

        def item(j, _):
            n = j // HPG
            i = j % HPG
            g = n % NG
            q = qt_s[n]
            q = jnp.where(rowhead == i, q, jnp.zeros_like(q))
            r16 = pl.ds(pl.multiple_of(i * Dh, Dh), Dh)

            def chunk(c, carry):
                m, l, a = carry
                ck = pl.ds(pl.multiple_of(c * _KX, _KX), _KX)
                s = jnp.dot(k_s[g, ck, :], q, preferred_element_type=_F32)
                mn = jnp.maximum(m, jnp.max(s, axis=0, keepdims=True))
                al = jnp.exp2(m - mn)
                p = jnp.exp2(s - mn)
                l = l * al + jnp.sum(p, axis=0, keepdims=True)
                a = a * al + jnp.dot(vt_s[g, r16, ck], p.astype(_BF),
                                     preferred_element_type=_F32)
                return mn, l, a
            m, l, a = lax.fori_loop(
                0, S // _KX, chunk,
                (jnp.full((1, _TQ), -jnp.inf, _F32), jnp.zeros((1, _TQ), _F32),
                 jnp.zeros((Dh, _TQ), _F32)))
            ot_s[n, r16, :] = (a * pl.reciprocal(l, approx=False)).astype(_BF)
            return 0
        lax.fori_loop(0, NT * _H, item, 0)

    for cp in cp_rest:
        cp.wait()

    def stage_x(r):
        t, u = divmod(r, _TQ // _TR)
        ot = ot_s[pl.ds(t * NG, NG), :, u * _TR:(u + 1) * _TR].reshape(D, _TR)
        a = lax.dot_general(ot, wo_s[...], (((0,), (0,)), ((), ())), preferred_element_type=_F32)
        x1 = x_s[rows(r, _TR), :].astype(_F32) + mod(2) * a
        h2 = (_layernorm(x1) * (1.0 + mod(4)) + mod(3)).astype(_BF)
        return x1, h2

    def stage_f1(h2):
        f = jnp.dot(h2, w1_s[...], preferred_element_type=_F32) + b1_s[...].astype(_F32)
        f = jnp.maximum(f, 0.0)
        return (f * f).astype(_BF)

    out_cp = []
    xs = {0: stage_x(0)}
    pend = {}
    for r in range(NR + 1):
        if r < NR:
            x1, h2 = xs.pop(r)
            f = stage_f1(h2)
            pend[r] = (x1, f)
        if r + 1 < NR:
            xs[r + 1] = stage_x(r + 1)
        if r >= 1:
            x1, f = pend.pop(r - 1)
            y = jnp.dot(f, w2_s[...], preferred_element_type=_F32) + b2_s[...].astype(_F32)
            out_s[rows(r - 1, _TR), :] = (x1 + mod(5) * y).astype(out_s.dtype)
            cp = pltpu.make_async_copy(out_s.at[rows(r - 1, _TR)], o_hbm.at[rows(r - 1, _TR)], osems.at[r - 1])
            cp.start()
            out_cp.append(cp)
    for cp in out_cp:
        cp.wait()


@jax.jit
def pallas_adaLN_cond__mha_block__dense_activation_squared_relu__prompt_kernel(
    A_x: jax.Array,
    A_wqkv: jax.Array,
    A_wo: jax.Array,
    B_x: jax.Array,
    B_w1: jax.Array,
    B_b1: jax.Array,
    B_w2: jax.Array,
    B_b2: jax.Array,
    c: jax.Array,
    w_mod: jax.Array,
):
    del B_x
    B, S, D = A_x.shape
    F = B_w1.shape[1]
    assert B == 1
    x2 = A_x.reshape(S, D)
    any_spec = pl.BlockSpec(memory_space=pl.ANY)
    out = pl.pallas_call(
        functools.partial(_kernel, S=S, D=D),
        in_specs=[any_spec] * 9,
        out_specs=any_spec,
        out_shape=jax.ShapeDtypeStruct((S, D), A_x.dtype),
        scratch_shapes=[
            pltpu.VMEM((S, D), A_x.dtype),
            pltpu.VMEM((3, D, D), A_wqkv.dtype),
            pltpu.VMEM((D, D), A_wo.dtype),
            pltpu.VMEM((D, F), B_w1.dtype),
            pltpu.VMEM((1, F), B_b1.dtype),
            pltpu.VMEM((F, D), B_w2.dtype),
            pltpu.VMEM((1, D), B_b2.dtype),
            pltpu.VMEM((1, D), c.dtype),
            pltpu.VMEM((3, D, 2 * D), w_mod.dtype),
            pltpu.VMEM((8, 6 * D), _F32),
            pltpu.VMEM((S // _TQ * D // _G, _G, _TQ), _BF),
            pltpu.VMEM((D // _G, S, _G), _BF),
            pltpu.VMEM((D // _G, _G, S), _BF),
            pltpu.VMEM((S // _TQ * D // _G, _G, _TQ), _BF),
            pltpu.VMEM((S, D), A_x.dtype),
            pltpu.SemaphoreType.DMA((12 + S // _TQ,)),
            pltpu.SemaphoreType.DMA((S // _TR,)),
        ],
        compiler_params=pltpu.CompilerParams(
            vmem_limit_bytes=110 * 1024 * 1024,
        ),
    )(x2, A_wqkv, A_wo, B_w1, B_b1.reshape(1, F), B_w2, B_b2.reshape(1, D), c, w_mod)
    return out.reshape(B, S, D)
```

```python
import functools

import jax
import jax.numpy as jnp
import numpy as np
from jax import lax
import jax.experimental.pallas as pl
import jax.experimental.pallas.tpu as pltpu

_BF = jnp.bfloat16
_F32 = jnp.float32
_LOG2E = float(np.log2(np.e))
_EPS = 1e-5

_H = 32
_TQ = 512
_TP = 256
_TR = 256
_KC = 128
_KX = 256
_G = 128


def _layernorm(x):
    m = jnp.mean(x, axis=-1, keepdims=True)
    xc = x - m
    v = jnp.mean(xc * xc, axis=-1, keepdims=True)
    return xc * lax.rsqrt(v + _EPS)


def _kernel(x_hbm, wqkv_hbm, wo_hbm, w1_hbm, b1_hbm, w2_hbm, b2_hbm, c_hbm, wmod_hbm,
            o_hbm,
            x_s, wqkv_s, wo_s, w1_s, b1_s, w2_s, b2_s, c_s, wmod_s, mod_s,
            qt_s, k_s, vt_s, ot_s, out_s, sems, osems, *, S, D):
    Dh = D // _H
    NT = S // _TQ
    NG = D // _G
    HPG = _G // Dh
    NC = S // _KC
    NR = S // _TR

    def rows(t, n):
        return pl.ds(t * n, n)

    cp_c = pltpu.make_async_copy(c_hbm, c_s, sems.at[0])
    cp_mod = [pltpu.make_async_copy(wmod_hbm.at[:, j * 2 * D:(j + 1) * 2 * D], wmod_s.at[j], sems.at[1 + j])
              for j in range(3)]
    cp_qkv = [pltpu.make_async_copy(wqkv_hbm.at[:, j * D:(j + 1) * D], wqkv_s.at[j], sems.at[4 + j])
              for j in range(3)]
    cp_x = [pltpu.make_async_copy(x_hbm.at[rows(t, S // 2)], x_s.at[rows(t, S // 2)], sems.at[7 + t])
            for t in range(2)]
    cp_rest = [
        pltpu.make_async_copy(wo_hbm, wo_s, sems.at[9]),
        pltpu.make_async_copy(w1_hbm, w1_s, sems.at[10]),
        pltpu.make_async_copy(b1_hbm, b1_s, sems.at[11]),
        pltpu.make_async_copy(w2_hbm, w2_s, sems.at[12]),
        pltpu.make_async_copy(b2_hbm, b2_s, sems.at[13]),
    ]

    def mod(j):
        return mod_s[0:1, j * D:(j + 1) * D]

    for cp in [cp_c, cp_mod[0], cp_x[0]] + cp_qkv:
        cp.start()
    cp_c.wait()
    cv = c_s[...].astype(_F32)
    sc = jnp.broadcast_to((cv * jax.nn.sigmoid(cv)).astype(_BF), (16, D))

    def modulation(j):
        mod_s[:, j * 2 * D:(j + 1) * 2 * D] = jnp.dot(
            sc, wmod_s[j], preferred_element_type=_F32)[0:8]

    cp_mod[0].wait()
    cp_x[0].wait()
    modulation(0)

    def ln1(t):
        xr = x_s[rows(t, _TP), :].astype(_F32)
        return (_layernorm(xr) * (1.0 + mod(1)) + mod(0)).astype(_BF)

    NP = S // _TP
    hn = ln1(0)
    for cp in cp_qkv:
        cp.wait()
    for cp in cp_x[1:] + cp_mod[1:] + cp_rest:
        cp.start()
    for t in range(NP):
        h = hn
        q = jnp.dot(h, wqkv_s[0], preferred_element_type=_F32)
        k = jnp.dot(h, wqkv_s[1], preferred_element_type=_F32)
        v = jnp.dot(h, wqkv_s[2], preferred_element_type=_F32)
        if t + 1 == NP // 2:
            cp_x[1].wait()
        if t + 1 < NP:
            hn = ln1(t + 1)
        tq, u = divmod(t, _TQ // _TP)
        q = q * (Dh ** -0.5 * _LOG2E)
        qt_s[pl.ds(tq * NG, NG), :, u * _TP:(u + 1) * _TP] = q.T.astype(_BF).reshape(NG, _G, _TP)
        k = k.astype(_BF)
        for g in range(NG):
            k_s[g, rows(t, _TP), :] = k[:, g * _G:(g + 1) * _G]
        vt = v.T.astype(_BF)
        for g in range(NG):
            vt_s[g, :, rows(t, _TP)] = vt[g * _G:(g + 1) * _G]
    cp_mod[1].wait()
    cp_mod[2].wait()
    modulation(1)
    modulation(2)

    def attn_body(n, carry):
        lmax, lmin = carry
        g = n % NG
        seq = [(i, c) for i in range(HPG) for c in range(NC)]
        qm, sv, pv, acc, l8 = {}, {}, {}, {}, {}
        for u in range(len(seq) + 2):
            if u < len(seq):
                i, c = seq[u]
                if c == 0:
                    parts = [qt_s[n, i * Dh:(i + 1) * Dh, :]]
                    if i > 0:
                        parts = [jnp.zeros((i * Dh, _TQ), _BF)] + parts
                    if i < HPG - 1:
                        parts = parts + [jnp.zeros((_G - (i + 1) * Dh, _TQ), _BF)]
                    qm[i] = jnp.concatenate(parts, axis=0)
                sv[u] = jnp.dot(k_s[g, c * _KC:(c + 1) * _KC, :], qm[i],
                                preferred_element_type=_F32)
            if 0 <= u - 1 < len(seq):
                i, c = seq[u - 1]
                s = sv.pop(u - 1)
                ps, ls = [], None
                for r in range(_KC // 16):
                    p = jnp.exp2(s[r * 16:(r + 1) * 16])
                    t2 = p[0:8] + p[8:16]
                    ls = t2 if ls is None else ls + t2
                    ps.append(p.astype(_BF))
                pv[u - 1] = jnp.concatenate(ps, axis=0)
                l8[i] = ls if c == 0 else l8[i] + ls
            if u - 2 >= 0:
                i, c = seq[u - 2]
                v = vt_s[g, i * Dh:(i + 1) * Dh, c * _KC:(c + 1) * _KC]
                r = jnp.dot(v, pv.pop(u - 2), preferred_element_type=_F32)
                acc[i] = r if c == 0 else acc[i] + r
                if c == NC - 1:
                    l = jnp.sum(l8[i], axis=0, keepdims=True)
                    lmax = jnp.maximum(lmax, l)
                    lmin = jnp.minimum(lmin, l)
                    o = acc[i] * pl.reciprocal(l, approx=False)
                    ot_s[n, i * Dh:(i + 1) * Dh, :] = o.astype(_BF)
        return lmax, lmin

    lmax, lmin = lax.fori_loop(
        0, NT * NG, attn_body,
        (jnp.ones((1, _TQ), _F32), jnp.ones((1, _TQ), _F32)))
    ok = jnp.logical_and(lmax <= 2.0 ** 100, lmin >= 2.0 ** -60)
    n_bad = jnp.sum(jnp.where(ok, 0.0, 1.0))

    @pl.when(n_bad > 0.0)
    def _exact_attention():
        rowhead = lax.broadcasted_iota(jnp.int32, (_G, _TQ), 0) // Dh

        def item(j, _):
            n = j // HPG
            i = j % HPG
            g = n % NG
            q = qt_s[n]
            q = jnp.where(rowhead == i, q, jnp.zeros_like(q))
            r16 = pl.ds(pl.multiple_of(i * Dh, Dh), Dh)

            def chunk(c, carry):
                m, l, a = carry
                ck = pl.ds(pl.multiple_of(c * _KX, _KX), _KX)
                s = jnp.dot(k_s[g, ck, :], q, preferred_element_type=_F32)
                mn = jnp.maximum(m, jnp.max(s, axis=0, keepdims=True))
                al = jnp.exp2(m - mn)
                p = jnp.exp2(s - mn)
                l = l * al + jnp.sum(p, axis=0, keepdims=True)
                a = a * al + jnp.dot(vt_s[g, r16, ck], p.astype(_BF),
                                     preferred_element_type=_F32)
                return mn, l, a
            m, l, a = lax.fori_loop(
                0, S // _KX, chunk,
                (jnp.full((1, _TQ), -jnp.inf, _F32), jnp.zeros((1, _TQ), _F32),
                 jnp.zeros((Dh, _TQ), _F32)))
            ot_s[n, r16, :] = (a * pl.reciprocal(l, approx=False)).astype(_BF)
            return 0
        lax.fori_loop(0, NT * _H, item, 0)

    for cp in cp_rest:
        cp.wait()

    def stage_x(r):
        t, u = divmod(r, _TQ // _TR)
        ot = ot_s[pl.ds(t * NG, NG), :, u * _TR:(u + 1) * _TR].reshape(D, _TR)
        a = lax.dot_general(ot, wo_s[...], (((0,), (0,)), ((), ())), preferred_element_type=_F32)
        x1 = x_s[rows(r, _TR), :].astype(_F32) + mod(2) * a
        h2 = (_layernorm(x1) * (1.0 + mod(4)) + mod(3)).astype(_BF)
        return x1, h2

    def stage_f1(h2):
        f = jnp.dot(h2, w1_s[...], preferred_element_type=_F32) + b1_s[...].astype(_F32)
        f = jnp.maximum(f, 0.0)
        return (f * f).astype(_BF)

    out_cp = []
    xs = {0: stage_x(0)}
    pend = {}
    for r in range(NR + 1):
        if r < NR:
            x1, h2 = xs.pop(r)
            f = stage_f1(h2)
            pend[r] = (x1, f)
        if r + 1 < NR:
            xs[r + 1] = stage_x(r + 1)
        if r >= 1:
            x1, f = pend.pop(r - 1)
            y = jnp.dot(f, w2_s[...], preferred_element_type=_F32) + b2_s[...].astype(_F32)
            out_s[rows(r - 1, _TR), :] = (x1 + mod(5) * y).astype(out_s.dtype)
            cp = pltpu.make_async_copy(out_s.at[rows(r - 1, _TR)], o_hbm.at[rows(r - 1, _TR)], osems.at[r - 1])
            cp.start()
            out_cp.append(cp)
    for cp in out_cp:
        cp.wait()


@jax.jit
def pallas_adaLN_cond__mha_block__dense_activation_squared_relu__prompt_kernel(
    A_x: jax.Array,
    A_wqkv: jax.Array,
    A_wo: jax.Array,
    B_x: jax.Array,
    B_w1: jax.Array,
    B_b1: jax.Array,
    B_w2: jax.Array,
    B_b2: jax.Array,
    c: jax.Array,
    w_mod: jax.Array,
):
    del B_x
    B, S, D = A_x.shape
    F = B_w1.shape[1]
    assert B == 1
    x2 = A_x.reshape(S, D)
    any_spec = pl.BlockSpec(memory_space=pltpu.HBM)
    out = pl.pallas_call(
        functools.partial(_kernel, S=S, D=D),
        in_specs=[any_spec] * 9,
        out_specs=any_spec,
        out_shape=jax.ShapeDtypeStruct((S, D), A_x.dtype),
        scratch_shapes=[
            pltpu.VMEM((S, D), A_x.dtype),
            pltpu.VMEM((3, D, D), A_wqkv.dtype),
            pltpu.VMEM((D, D), A_wo.dtype),
            pltpu.VMEM((D, F), B_w1.dtype),
            pltpu.VMEM((1, F), B_b1.dtype),
            pltpu.VMEM((F, D), B_w2.dtype),
            pltpu.VMEM((1, D), B_b2.dtype),
            pltpu.VMEM((1, D), c.dtype),
            pltpu.VMEM((3, D, 2 * D), w_mod.dtype),
            pltpu.VMEM((8, 6 * D), _F32),
            pltpu.VMEM((S // _TQ * D // _G, _G, _TQ), _BF),
            pltpu.VMEM((D // _G, S, _G), _BF),
            pltpu.VMEM((D // _G, _G, S), _BF),
            pltpu.VMEM((S // _TQ * D // _G, _G, _TQ), _BF),
            pltpu.VMEM((S, D), A_x.dtype),
            pltpu.SemaphoreType.DMA((14,)),
            pltpu.SemaphoreType.DMA((S // _TR,)),
        ],
        compiler_params=pltpu.CompilerParams(
            vmem_limit_bytes=110 * 1024 * 1024,
        ),
    )(x2, A_wqkv, A_wo, B_w1, B_b1.reshape(1, F), B_w2, B_b2.reshape(1, D), c, w_mod)
    return out.reshape(B, S, D)
```

```python
import functools

import jax
import jax.numpy as jnp
import numpy as np
from jax import lax
import jax.experimental.pallas as pl
import jax.experimental.pallas.tpu as pltpu

_BF = jnp.bfloat16
_F32 = jnp.float32
_LOG2E = float(np.log2(np.e))
_EPS = 1e-5

_H = 32
_TQ = 512
_TP = 256
_TR = 128
_LO = 2
_KC = 128
_KX = 256
_GU = 2
_G = 128


def _layernorm(x):
    m = jnp.mean(x, axis=-1, keepdims=True)
    xc = x - m
    v = jnp.mean(xc * xc, axis=-1, keepdims=True)
    return xc * lax.rsqrt(v + _EPS)


def _kernel(x_hbm, wqkv_hbm, wo_hbm, w1_hbm, b1_hbm, w2_hbm, b2_hbm, c_hbm, wmod_hbm,
            o_hbm,
            x_s, wqkv_s, wo_s, w1_s, b1_s, w2_s, b2_s, c_s, wmod_s, mod_s,
            qt_s, k_s, vt_s, ot_s, out_s, sems, osems, *, S, D):
    Dh = D // _H
    NT = S // _TQ
    NG = D // _G
    HPG = _G // Dh
    NC = S // _KC
    NR = S // _TR

    def rows(t, n):
        return pl.ds(t * n, n)

    cp_c = pltpu.make_async_copy(c_hbm, c_s, sems.at[0])
    cp_mod = [pltpu.make_async_copy(wmod_hbm.at[:, j * D:(j + 1) * D], wmod_s.at[j], sems.at[1 + j])
              for j in range(6)]
    cp_qkv = [pltpu.make_async_copy(wqkv_hbm.at[:, j * D:(j + 1) * D], wqkv_s.at[j], sems.at[14 + j])
              for j in range(3)]
    xsplit = [0, 2 * _TP, S // 2, S]
    cp_x = [pltpu.make_async_copy(x_hbm.at[xsplit[t]:xsplit[t + 1]], x_s.at[xsplit[t]:xsplit[t + 1]], sems.at[17 + t])
            for t in range(3)]
    cp_rest = [
        pltpu.make_async_copy(wo_hbm, wo_s, sems.at[9]),
        pltpu.make_async_copy(w1_hbm, w1_s, sems.at[10]),
        pltpu.make_async_copy(b1_hbm, b1_s, sems.at[11]),
        pltpu.make_async_copy(w2_hbm, w2_s, sems.at[12]),
        pltpu.make_async_copy(b2_hbm, b2_s, sems.at[13]),
    ]

    def mod(j):
        return mod_s[0:1, j * D:(j + 1) * D]

    for cp in [cp_c, cp_mod[0], cp_mod[1], cp_x[0], cp_qkv[0], cp_x[1], cp_qkv[1], cp_qkv[2]]:
        cp.start()
    cp_c.wait()
    cv = c_s[...].astype(_F32)
    sc = jnp.broadcast_to((cv * jax.nn.sigmoid(cv)).astype(_BF), (16, D))

    def modulation(j):
        mod_s[:, j * D:(j + 1) * D] = jnp.dot(
            sc, wmod_s[j], preferred_element_type=_F32)[0:8]

    cp_mod[0].wait()
    cp_mod[1].wait()
    modulation(0)
    modulation(1)
    cp_x[0].wait()

    def ln1(t):
        xr = x_s[rows(t, _TP), :].astype(_F32)
        return (_layernorm(xr) * (1.0 + mod(1)) + mod(0)).astype(_BF)

    NP = S // _TP

    def epi_q(t, q):
        tq, u = divmod(t, _TQ // _TP)
        q = q * (Dh ** -0.5 * _LOG2E)
        qt_s[pl.ds(tq * NG, NG), :, u * _TP:(u + 1) * _TP] = q.T.astype(_BF).reshape(NG, _G, _TP)

    def epi_k(t, k):
        k = k.astype(_BF)
        for g in range(NG):
            k_s[g, rows(t, _TP), :] = k[:, g * _G:(g + 1) * _G]

    def epi_v(t, v):
        vt = v.T.astype(_BF)
        for g in range(NG):
            vt_s[g, :, rows(t, _TP)] = vt[g * _G:(g + 1) * _G]

    def proj(h, j):
        return jnp.dot(h, wqkv_s[j], preferred_element_type=_F32)

    NE = NP // 2
    hs = {0: ln1(0), 1: ln1(1)}
    cp_qkv[0].wait()
    qv = {0: proj(hs[0], 0)}
    cp_x[1].wait()
    qv[1] = proj(hs[1], 0)
    hs[2] = ln1(2)
    epi_q(0, qv.pop(0))
    qv[2] = proj(hs[2], 0)
    hs[3] = ln1(3)
    epi_q(1, qv.pop(1))
    qv[3] = proj(hs[3], 0)
    epi_q(2, qv.pop(2))
    cp_qkv[1].wait()
    cp_qkv[2].wait()
    for cp in cp_x[2:] + cp_mod[2:] + cp_rest:
        cp.start()
    prev = (epi_q, 3, qv.pop(3))
    for j, e in ((1, epi_k), (2, epi_v)):
        for t in range(NE):
            if j == 2 and t == NE - 1:
                cp_x[2].wait()
            r = proj(hs[t], j)
            prev[0](*prev[1:])
            prev = (e, t, r)
    hn = ln1(NE)
    prev = [prev]
    for t in range(NE, NP):
        h = hn
        q, k, v = proj(h, 0), proj(h, 1), proj(h, 2)
        for e, tt, r in prev:
            e(tt, r)
        if t + 1 < NP:
            hn = ln1(t + 1)
        prev = [(epi_q, t, q), (epi_k, t, k), (epi_v, t, v)]
    for j in range(2, 6):
        cp_mod[j].wait()
    for j in range(2, 6):
        modulation(j)
    for e, tt, r in prev:
        e(tt, r)

    def attn_body(it, carry):
        lmax, lmin, bad8 = carry
        seq = [(j, i, c) for j in range(_GU) for i in range(HPG) for c in range(NC)]
        qm, sv, pv, acc, l8 = {}, {}, {}, {}, {}

        def unit(j):
            n = it * _GU + j
            g = n % NG if _GU % NG else j % NG
            return n, g

        for u in range(len(seq) + 2):
            if u < len(seq):
                j, i, c = seq[u]
                n, g = unit(j)
                if c == 0:
                    parts = [qt_s[n, i * Dh:(i + 1) * Dh, :]]
                    if i > 0:
                        parts = [jnp.zeros((i * Dh, _TQ), _BF)] + parts
                    if i < HPG - 1:
                        parts = parts + [jnp.zeros((_G - (i + 1) * Dh, _TQ), _BF)]
                    qm[j, i] = jnp.concatenate(parts, axis=0)
                sv[u] = jnp.dot(k_s[g, c * _KC:(c + 1) * _KC, :], qm[j, i],
                                preferred_element_type=_F32)
            if 0 <= u - 1 < len(seq):
                j, i, c = seq[u - 1]
                s = sv.pop(u - 1)
                ps, ls = [], None
                for r in range(_KC // 16):
                    p = jnp.exp2(s[r * 16:(r + 1) * 16])
                    t2 = p[0:8] + p[8:16]
                    ls = t2 if ls is None else ls + t2
                    ps.append(p.astype(_BF))
                pv[u - 1] = jnp.concatenate(ps, axis=0)
                l8[j, i] = ls if c == 0 else l8[j, i] + ls
            if u - 2 >= 0:
                j, i, c = seq[u - 2]
                n, g = unit(j)
                v = vt_s[g, i * Dh:(i + 1) * Dh, c * _KC:(c + 1) * _KC]
                r = jnp.dot(v, pv.pop(u - 2), preferred_element_type=_F32)
                acc[j, i] = r if c == 0 else acc[j, i] + r
                if c == NC - 1:
                    l = jnp.sum(l8.pop((j, i)), axis=0, keepdims=True)
                    lmax = jnp.maximum(lmax, l)
                    lmin = jnp.minimum(lmin, l)
                    a = acc.pop((j, i))
                    b = jnp.where(jnp.abs(a) < 2.0 ** 126, 0.0, 1.0)
                    bad8 = jnp.maximum(bad8, jnp.maximum(b[0:8], b[8:16]))
                    o = a * pltpu.reciprocal(l, approx=False)
                    ot_s[n, i * Dh:(i + 1) * Dh, :] = o.astype(_BF)
        return lmax, lmin, bad8

    lmax, lmin, bad8 = lax.fori_loop(
        0, NT * NG // _GU, attn_body,
        (jnp.ones((1, _TQ), _F32), jnp.ones((1, _TQ), _F32), jnp.zeros((8, _TQ), _F32)))
    ok = jnp.logical_and(lmax <= 2.0 ** 100, lmin >= 2.0 ** -30)
    n_bad = jnp.sum(jnp.where(ok, 0.0, 1.0)) + jnp.sum(bad8)

    @pl.when(n_bad > 0.0)
    def _exact_attention():
        rowhead = lax.broadcasted_iota(jnp.int32, (_G, _TQ), 0) // Dh

        def item(j, _):
            n = j // HPG
            i = j % HPG
            g = n % NG
            q = qt_s[n]
            q = jnp.where(rowhead == i, q, jnp.zeros_like(q))
            r16 = pl.ds(pl.multiple_of(i * Dh, Dh), Dh)

            def chunk(c, carry):
                m, l, a = carry
                ck = pl.ds(pl.multiple_of(c * _KX, _KX), _KX)
                s = jnp.dot(k_s[g, ck, :], q, preferred_element_type=_F32)
                mn = jnp.maximum(m, jnp.max(s, axis=0, keepdims=True))
                al = jnp.exp2(m - mn)
                p = jnp.exp2(s - mn)
                l = l * al + jnp.sum(p, axis=0, keepdims=True)
                a = a * al + jnp.dot(vt_s[g, r16, ck], p.astype(_BF),
                                     preferred_element_type=_F32)
                return mn, l, a
            m, l, a = lax.fori_loop(
                0, S // _KX, chunk,
                (jnp.full((1, _TQ), -jnp.inf, _F32), jnp.zeros((1, _TQ), _F32),
                 jnp.zeros((Dh, _TQ), _F32)))
            ot_s[n, r16, :] = (a * pltpu.reciprocal(l, approx=False)).astype(_BF)
            return 0
        lax.fori_loop(0, NT * _H, item, 0)

    for cp in cp_rest:
        cp.wait()

    def stage_o(r):
        t, u = divmod(r, _TQ // _TR)
        ot = ot_s[pl.ds(t * NG, NG), :, u * _TR:(u + 1) * _TR].reshape(D, _TR)
        return lax.dot_general(ot, wo_s[...], (((0,), (0,)), ((), ())), preferred_element_type=_F32)

    def stage_ln(r, a):
        x1 = x_s[rows(r, _TR), :].astype(_F32) + mod(2) * a
        h2 = (_layernorm(x1) * (1.0 + mod(4)) + mod(3)).astype(_BF)
        return x1, h2

    def stage_f1(h2):
        f = jnp.dot(h2, w1_s[...], preferred_element_type=_F32) + b1_s[...].astype(_F32).reshape(1, -1)
        f = jnp.maximum(f, 0.0)
        return (f * f).astype(_BF)

    out_cp = []
    av = {r: stage_o(r) for r in range(_LO)}
    xs = {0: stage_ln(0, av.pop(0))}
    pend = {}
    for r in range(NR + 1):
        if r < NR:
            x1, h2 = xs.pop(r)
            f = stage_f1(h2)
            pend[r] = (x1, f)
        if r + _LO < NR:
            av[r + _LO] = stage_o(r + _LO)
        if r + 1 < NR:
            xs[r + 1] = stage_ln(r + 1, av.pop(r + 1))
        if r >= 1:
            x1, f = pend.pop(r - 1)
            y = jnp.dot(f, w2_s[...], preferred_element_type=_F32) + b2_s[...].astype(_F32).reshape(1, -1)
            out_s[rows(r - 1, _TR), :] = (x1 + mod(5) * y).astype(out_s.dtype)
            cp = pltpu.make_async_copy(out_s.at[rows(r - 1, _TR)], o_hbm.at[rows(r - 1, _TR)], osems.at[r - 1])
            cp.start()
            out_cp.append(cp)
    for cp in out_cp:
        cp.wait()


@jax.jit
def pallas_adaLN_cond__mha_block__dense_activation_squared_relu__prompt_kernel(
    A_x: jax.Array,
    A_wqkv: jax.Array,
    A_wo: jax.Array,
    B_x: jax.Array,
    B_w1: jax.Array,
    B_b1: jax.Array,
    B_w2: jax.Array,
    B_b2: jax.Array,
    c: jax.Array,
    w_mod: jax.Array,
):
    del B_x
    B, S, D = A_x.shape
    F = B_w1.shape[1]
    assert B == 1 and S == 8 * _TP and D == _H * 16 and D % _G == 0
    x2 = A_x.reshape(S, D)
    any_spec = pl.BlockSpec(memory_space=pltpu.HBM)
    out = pl.pallas_call(
        functools.partial(_kernel, S=S, D=D),
        in_specs=[any_spec] * 9,
        out_specs=any_spec,
        out_shape=jax.ShapeDtypeStruct((S, D), A_x.dtype),
        scratch_shapes=[
            pltpu.VMEM((S, D), A_x.dtype),
            pltpu.VMEM((3, D, D), A_wqkv.dtype),
            pltpu.VMEM((D, D), A_wo.dtype),
            pltpu.VMEM((D, F), B_w1.dtype),
            pltpu.VMEM((F,), B_b1.dtype),
            pltpu.VMEM((F, D), B_w2.dtype),
            pltpu.VMEM((D,), B_b2.dtype),
            pltpu.VMEM((1, D), c.dtype),
            pltpu.VMEM((6, D, D), w_mod.dtype),
            pltpu.VMEM((8, 6 * D), _F32),
            pltpu.VMEM((S // _TQ * D // _G, _G, _TQ), _BF),
            pltpu.VMEM((D // _G, S, _G), _BF),
            pltpu.VMEM((D // _G, _G, S), _BF),
            pltpu.VMEM((S // _TQ * D // _G, _G, _TQ), _BF),
            pltpu.VMEM((S, D), A_x.dtype),
            pltpu.SemaphoreType.DMA((20,)),
            pltpu.SemaphoreType.DMA((S // _TR,)),
        ],
        compiler_params=pltpu.CompilerParams(
            vmem_limit_bytes=110 * 1024 * 1024,
        ),
    )(x2, A_wqkv, A_wo, B_w1, B_b1, B_w2, B_b2, c, w_mod)
    return out.reshape(B, S, D)
```
